```python
import os as _os
_os.environ.setdefault('JAX_PLATFORMS', 'cpu')
import jax
import jax.numpy as jnp

def _softmax(x, axis=-1):
    return jax.nn.softmax(x, axis=axis)

def _gelu(x):
    return jax.nn.gelu(x, approximate=True)

def _silu(x):
    return jax.nn.silu(x)

def _sigmoid(x):
    return jax.nn.sigmoid(x)

def _layernorm(x, axis=-1, eps=1e-05):
    m = jnp.mean(x, axis=axis, keepdims=True)
    v = jnp.var(x, axis=axis, keepdims=True)
    return (x - m) / jnp.sqrt(v + eps)

def _scatter_add(tgt, idx, src, axis=0):
    return tgt.at[idx].add(src)

def _segment_sum(src, seg, n):
    return jax.ops.segment_sum(src, seg, n)

class _Rng:

    def __init__(self, key):
        self._k = key

    def _next(self):
        self._k, sub = jax.random.split(self._k)
        return sub

    def normal(self, shape):
        return jax.random.normal(self._next(), shape, dtype=jnp.bfloat16)

    def randint(self, lo, hi, shape):
        return jax.random.randint(self._next(), shape, lo, hi, dtype=jnp.int32)

    def uniform(self, shape, lo=0.0, hi=1.0):
        return jax.random.uniform(self._next(), shape, jnp.bfloat16, lo, hi)

    def permutation(self, n):
        return jax.random.permutation(self._next(), n)
kernel_name = 'standalone__conformer_family_e_branchformer__speech'

def setup_inputs():
    _rng = _Rng(jax.random.key(int.from_bytes(__import__("os").urandom(4), "little")))
    _w = lambda a: (lambda t: t.astype(jnp.bfloat16) if jnp.issubdtype(t.dtype, jnp.floating) else t)(jnp.asarray(a))
    B, T, D, K = (2, 4000, 256, 31)
    return {'x': _w((lambda *s: _rng.normal(s) * 0.05)(B, T, D)), 'w_qkv': _w((lambda *s: _rng.normal(s) * 0.05)(D, 3 * D)), 'w_att_out': _w((lambda *s: _rng.normal(s) * 0.05)(D, D)), 'w_mlp_in': _w((lambda *s: _rng.normal(s) * 0.05)(D, 2 * D)), 'dw_csgu': _w((lambda *s: _rng.normal(s) * 0.05)(K, D)), 'w_mlp_out': _w((lambda *s: _rng.normal(s) * 0.05)(D, D)), 'dw_merge': _w((lambda *s: _rng.normal(s) * 0.05)(K, 2 * D)), 'w_merge': _w((lambda *s: _rng.normal(s) * 0.05)(2 * D, D))}

def reference(x, w_qkv, w_att_out, w_mlp_in, dw_csgu, w_mlp_out, dw_merge, w_merge):
    B, T, D = x.shape
    K = dw_csgu.shape[0]
    pad = K // 2
    xa = _layernorm(x, axis=-1)
    qkv = jnp.einsum('btd,de->bte', xa, w_qkv)
    q, k, v = (qkv[..., :D].copy(), qkv[..., D:2 * D].copy(), qkv[..., 2 * D:].copy())
    scores = jnp.einsum('btd,bsd->bts', q, k) * D ** (-0.5)
    p = _softmax(scores, axis=-1)
    attn = jnp.einsum('bts,bsd->btd', p, v)
    glob = jnp.einsum('btd,de->bte', attn, w_att_out)
    xc = _layernorm(x, axis=-1)
    h = _gelu(jnp.einsum('btd,de->bte', xc, w_mlp_in))
    u, g = (h[..., :D].copy(), h[..., D:].copy())
    g = _layernorm(g, axis=-1)
    gp = jnp.pad(g, ((0, 0), (pad, pad), (0, 0)))
    gc = jnp.zeros_like(g)
    for i in range(K):
        gc = gc + gp[:, i:i + T, :] * dw_csgu[i][None, None, :]
    loc = jnp.einsum('btd,de->bte', u * gc, w_mlp_out)
    m = jnp.concatenate([glob, loc], axis=-1)
    mp = jnp.pad(m, ((0, 0), (pad, pad), (0, 0)))
    mc = jnp.zeros_like(m)
    for i in range(K):
        mc = mc + mp[:, i:i + T, :] * dw_merge[i][None, None, :]
    m = m + mc
    return x + jnp.einsum('btc,cd->btd', m, w_merge)
```

```python
import functools
import math
import os

import jax
import jax.numpy as jnp
from jax import lax
import jax.experimental.pallas as pl
import jax.experimental.pallas.tpu as pltpu

F32 = jnp.float32
BF16 = jnp.bfloat16
U32 = jnp.uint32

TQ = 400
TL = 512
TK = int(os.environ.get("TK", "256"))
HALO = 16
MINI = 32
LD = TQ // 8
LE = (TQ - MINI) // 8
LOG2E = math.log2(math.e)
NBLK = 8
RC = int(os.environ.get("RC", "200"))
EPARTS = int(os.environ.get("EPARTS", "2"))
DPARTS = int(os.environ.get("DPARTS", "1"))
FEND = int(os.environ.get("FEND", "0"))
XW = [int(v) for v in os.environ.get("XW", "0,1,3").split(",")]
ALAG = int(os.environ.get("ALAG", "3"))
S0ORD = int(os.environ.get("S0ORD", "0"))
PNOP = int(os.environ.get("PNOP", "3000"))


def _ln(xf, eps=1e-5):
    mu = jnp.mean(xf, axis=-1, keepdims=True)
    xc = xf - mu
    var = jnp.mean(xc * xc, axis=-1, keepdims=True)
    return xc * lax.rsqrt(var + eps)


def _gelu(x):
    c0 = math.sqrt(2.0 / math.pi)
    inner = x * (c0 + (c0 * 0.044715) * (x * x))
    hx = 0.5 * x
    return hx + hx * jnp.tanh(inner)


def _dot(a, b):
    return jnp.dot(a, b, preferred_element_type=F32)


def _dot_nt(a, b):
    return lax.dot_general(a, b, (((1,), (1,)), ((), ())), preferred_element_type=F32)


def _cat(planes):
    return jnp.concatenate(planes, axis=-1) if len(planes) > 1 else planes[0]


def _pk(v):
    return pltpu.bitcast(v, U32)


def _up(v):
    return pltpu.bitcast(v, BF16)


def _split_even(n, parts):
    out, o = [], 0
    for i in range(parts):
        e = ((n * (i + 1)) // parts) // 2 * 2 if i < parts - 1 else n
        out.append((o, e))
        o = e
    return out


def _kernel(x_hbm, wqkv_hbm, wo_hbm, win_hbm, dwc_hbm, wout_hbm, dwm_hbm, wm_hbm,
            o_hbm,
            x_ref, o_ref, wqkv_ref, wo_ref, win_ref, dwc_ref, wout_ref, dwm_ref, wm_ref,
            xa_buf, s_buf, mx_buf, u_buf, g_buf, m_buf, wqk, wvo, win, wout, wmg, wcb, wmb,
            ext_g, ext_m, q_buf, q_cur, a_buf, yst, yst2, sem_x, sem_w, sem_o, sc_ref,
            *, B, T, D, K):
    NQ = T // TQ
    NT = B * NQ
    TP = 2 * xa_buf.shape[1]
    TB = T + 2 * HALO
    NC = TP // TK
    NL = TP // TL
    PADK = K // 2
    M8 = MINI // 8

    xgroups = [(XW[i], (XW + [NL])[i + 1]) for i in range(len(XW))]

    def x_copy(b, l0, l1, si):
        g0 = b * T + l0 * TL
        n = min(l1 * TL, T) - l0 * TL
        return pltpu.make_async_copy(x_hbm.at[pl.ds(g0, n), :], x_ref.at[pl.ds(g0, n), :], sem_x.at[si])

    x0_copies = [x_copy(0, l0, l1, i) for i, (l0, l1) in enumerate(xgroups)]
    xr_copies = [x_copy(b, 0, NL, len(xgroups) + b - 1) for b in range(1, B)]

    wlist = [("qk", wqkv_hbm.at[:, pl.ds(0, 2 * D)], wqkv_ref.at[:, pl.ds(0, 2 * D)]),
             ("v", wqkv_hbm.at[:, pl.ds(2 * D, D)], wqkv_ref.at[:, pl.ds(2 * D, D)]),
             ("o", wo_hbm, wo_ref), ("dwc", dwc_hbm, dwc_ref),
             ("dwm", dwm_hbm, dwm_ref), ("in", win_hbm, win_ref), ("out", wout_hbm, wout_ref),
             ("mg", wm_hbm, wm_ref)]
    wcopy = {name: pltpu.make_async_copy(src, dst, sem_w.at[i]) for i, (name, src, dst) in enumerate(wlist)}

    def o_copy(g0, n, i):
        return pltpu.make_async_copy(o_ref.at[pl.ds(g0, n), :], o_hbm.at[pl.ds(g0, n), :], sem_o.at[i])

    x0_copies[0].start()
    wcopy["qk"].start()
    x0_copies[1].start()
    wcopy["in"].start()
    wcopy["dwc"].start()
    for cp in x0_copies[2:]:
        cp.start()
    for name in ("out", "v", "o", "dwm", "mg"):
        wcopy[name].start()

    sc_ref[0] = 0
    sc_ref[1] = 1

    for b in range(B):
        xa_buf[b, T // 2:TP // 2, :] = jnp.zeros(((TP - T) // 2, D), U32)
        for ct in range(2):
            g_buf[ct, b * TB:b * TB + HALO, :] = jnp.zeros((HALO, 128), F32)
            g_buf[ct, b * TB + HALO + T:(b + 1) * TB, :] = jnp.zeros((HALO, 128), F32)
        for ct in range(4):
            m_buf[ct, b * TB:b * TB + HALO, :] = jnp.zeros((HALO, 128), F32)
            m_buf[ct, b * TB + HALO + T:(b + 1) * TB, :] = jnp.zeros((HALO, 128), F32)

    def batch_of(v, per):
        if isinstance(v, int):
            return v // per
        return sum((v >= per * k).astype(jnp.int32) for k in range(1, B))

    def mo(v, m):
        return v if isinstance(v, int) else pl.multiple_of(v, m)

    def tile_pos(n):
        b = batch_of(n, NQ)
        return b, mo((n - b * NQ) * TQ, 16)

    def ln_rows(b, l):
        r0 = l * TL
        return b * T + r0, r0, min(TL, T - r0)

    def ln_chunk(b, l):
        g0, r0, n = ln_rows(b, l)
        xa = _ln(x_ref[g0:g0 + n, :].astype(F32)).astype(BF16)
        xa_buf[b, r0 // 2:(r0 + n) // 2, :] = _pk(xa)
        return xa

    def q_chunk(b, l, xa):
        g0, r0, n = ln_rows(b, l)
        q_buf[g0 // 2:(g0 + n) // 2, :] = _pk(_dot(xa, _up(wqk[...])).astype(BF16))

    def lnq_chunk(b, l):
        q_chunk(b, l, ln_chunk(b, l))

    def xa_rows(b, start, size):
        half = start // 2 if isinstance(start, int) else pl.multiple_of(lax.shift_right_logical(start, 1), 8)
        return _up(xa_buf[b, pl.ds(half, size // 2), :])

    def conv_nat(buf, ct, base, R, wb_ref, wct):
        acc = None
        for p in range(8):
            taps = list(range(p, K, 8))
            X = buf[ct, pl.ds(base - PADK + p, R + 8 * (len(taps) - 1)), :]
            X = X.reshape(-1, 8, 128)
            for k, i in enumerate(taps):
                w = wb_ref[i, :, wct * 128:(wct + 1) * 128]
                term = X[k:k + R // 8] * w[None]
                acc = term if acc is None else acc + term
        return acc.reshape(R, 128)

    def relayout(ext, ect, buf, ct, base, L):
        for e in range(L + K - 1):
            ext[ect, e * 8:(e + 1) * 8, :] = buf[ct, pl.ds(base - PADK + e, 8, stride=L), :]

    def conv_ext(ext, ect, j0, n, wb_ref, wct):
        X = ext[ect, j0 * 8:(j0 + n + K - 1) * 8, :].reshape(-1, 8, 128)
        acc = None
        for i in range(K):
            w = wb_ref[i, :, wct * 128:(wct + 1) * 128]
            term = X[i:i + n] * w[None]
            acc = term if acc is None else acc + term
        return acc.reshape(n * 8, 128)

    def conv_ext_dup(ext, ect, j0, n, wb_ref, wct, wct2):
        return jnp.concatenate(
            [conv_ext(ext, ect, j, 2, wb_ref, wct if (j // 2) % 2 == 0 else wct2)
             for j in range(j0, j0 + n, 2)], axis=0)

    def stage_A_q(n):
        q_cur[...] = q_buf[pl.ds(mo(n * (TQ // 2), 8), TQ // 2), :]

    def stage_A_chunk(n, c, mrun):
        b, _ = tile_pos(n)
        s = _dot_nt(_up(q_cur[...]), xa_rows(b, c * TK, TK))
        for l in range(TK // 128):
            sl = s[:, l * 128:(l + 1) * 128]
            k0 = c * TK + l * 128
            if k0 + 128 > T:
                lane = lax.broadcasted_iota(jnp.int32, (TQ, 128), 1)
                sl = jnp.where(lane < T - k0, sl, -jnp.inf)
            s_buf[:, k0:k0 + 128] = sl
            mrun = sl if mrun is None else jnp.maximum(mrun, sl)
        return mrun

    def stage_A_fin(mrun):
        mx = jnp.max(mrun, axis=-1, keepdims=True)
        mx_buf[...] = jnp.broadcast_to(mx, (TQ, 128))

    def stage_B_chunk(n, c, acc, lsum):
        b, _ = tile_pos(n)
        mx = mx_buf[...]
        p = jnp.exp2(s_buf[:, c * TK:(c + 1) * TK] - _cat([mx] * (TK // 128)))
        for l in range(TK // 128):
            pl_ = p[:, l * 128:(l + 1) * 128]
            lsum = pl_ if lsum is None else lsum + pl_
        d = _dot(p.astype(BF16), xa_rows(b, c * TK, TK))
        acc = d if acc is None else acc + d
        return acc, lsum

    def stage_B_fin(acc, lsum):
        l = jnp.sum(lsum, axis=-1, keepdims=True)
        a_buf[...] = _pk((acc * (1.0 / l)).astype(BF16))

    def items_G(n):
        def f():
            b, r0 = tile_pos(n)
            glob = _dot(_up(a_buf[...]), _up(wvo[...]))
            base = mo(b * TB + HALO + r0, 16)
            for ct in range(2):
                m_buf[ct, pl.ds(base, TQ), :] = glob[:, ct * 128:(ct + 1) * 128]
        return [(0, f)]

    def items_C(n):
        b, r0 = tile_pos(n)
        g0 = mo(n * TQ, 16)
        base = mo(b * TB + HALO + r0, 16)
        items = []
        splits = []
        o = 0
        while o < TQ:
            r = min(RC if (RC % 16 == 0) else (RC + 8 if (o // RC) % 2 == 0 else RC - 8), TQ - o)
            splits.append((o, r))
            o += r
        for (o, R) in splits:
            def f(o=o, R=R):
                h = _gelu(_dot(xa_rows(b, r0 + o, R), _up(win[...])))
                g = _ln(h[:, D:])
                for ct in range(2):
                    u_buf[ct, pl.ds(g0 + o, R), :] = h[:, ct * 128:(ct + 1) * 128]
                    g_buf[ct, pl.ds(base + o, R), :] = g[:, ct * 128:(ct + 1) * 128]
            items.append((R // 8 * 4 * 12, f))
        return items

    def items_D(n):
        b, r0 = tile_pos(n)
        base = mo(b * TB + HALO + r0, 16)
        g0 = mo(n * TQ, 16)
        L = LD
        items = []
        res = {}
        for ct in range(2):
            items.append((80, functools.partial(relayout, ext_g, ct, g_buf, ct, base, L)))
        for (p0, p1) in _split_even(L, DPARTS):
            for j0 in range(p0, p1, NBLK):
                n_ = min(NBLK, p1 - j0)
                for ct in range(2):
                    def f(j0=j0, n_=n_, ct=ct):
                        gc = conv_ext_dup(ext_g, ct, j0, n_, wcb, ct, ct + 2)
                        u = jnp.concatenate(
                            [u_buf[ct, pl.ds(g0 + j, 8, stride=L), :] for j in range(j0, j0 + n_)], axis=0)
                        res[j0, ct] = u * gc
                    items.append((n_ * 64, f))

            def fin(p0=p0, p1=p1):
                z = _cat([jnp.concatenate([res[j0, ct] for j0 in range(p0, p1, NBLK)], axis=0)
                          for ct in range(2)]).astype(BF16)
                loc = _dot(z, _up(wout[...]))
                for j in range(p0, p1):
                    for ct in range(2):
                        m_buf[2 + ct, pl.ds(base + j, 8, stride=L), :] = (
                            loc[(j - p0) * 8:(j - p0 + 1) * 8, ct * 128:(ct + 1) * 128])
            items.append((100, fin))
        return items

    def items_M(n, half, last=False):
        b, r0 = tile_pos(n)
        g0 = mo(n * TQ, 16)
        gp = max(n * TQ - MINI, 0) if isinstance(n, int) else pl.multiple_of(jnp.maximum(n * TQ - MINI, 0), 16)
        base_p = gp + HALO + batch_of(gp, T) * 2 * HALO
        base = b * TB + HALO + r0
        L = LE
        cts = (2 * half, 2 * half + 1)
        stage = yst if half else yst2
        items = []
        res = {}
        for ct in cts:
            items.append((80, functools.partial(relayout, ext_m, ct, m_buf, ct, base, L)))
        for ct in cts:
            def f(ct=ct):
                res[0, ct] = conv_nat(m_buf, ct, base_p, MINI, wmb, ct)
            items.append((M8 * 63, f))
        parts = _split_even(M8 + L, EPARTS)
        for (p0, p1) in parts:
            for j0 in range(max(p0, M8), p1, NBLK):
                n_ = min(NBLK, p1 - j0)
                for ct in cts:
                    def f(j0=j0, n_=n_, ct=ct):
                        res[j0, ct] = conv_ext_dup(ext_m, ct, j0 - M8, n_, wmb, ct, ct + 4)
                    items.append((n_ * 63, f))
            tail = last and p1 == M8 + L
            if tail:
                for ct in cts:
                    def f(ct=ct):
                        res[M8 + L, ct] = conv_nat(m_buf, ct, base + TQ - MINI, MINI, wmb, ct)
                    items.append((M8 * 63, f))

            def fin(p0=p0, p1=p1, tail=tail):
                js = ([0] if p0 == 0 else []) + list(range(max(p0, M8), p1, NBLK))
                if tail:
                    js.append(M8 + L)
                mm = _cat([jnp.concatenate([res[j0, ct] for j0 in js], axis=0)
                           for ct in cts]).astype(BF16)
                y = _dot(mm, _up(wmg[half * (D // 2):(half + 1) * (D // 2), :]))

                def nat(yrows, r, gdst):
                    if half:
                        for ct in range(2):
                            yst[ct, r:r + MINI, :] = yrows[:, ct * 128:(ct + 1) * 128]
                    else:
                        prev = _cat([yst[ct, r:r + MINI, :] for ct in range(2)])
                        o_ref[pl.ds(gdst, MINI), :] = (
                            x_ref[pl.ds(gdst, MINI), :].astype(F32) + prev + yrows).astype(BF16)
                if p0 == 0:
                    nat(y[:MINI], 0, gp)
                for j in range(max(p0, M8), p1):
                    for ct in range(2):
                        stage[ct, pl.ds(MINI + j - M8, 8, stride=L), :] = (
                            y[(j - p0) * 8:(j - p0 + 1) * 8, ct * 128:(ct + 1) * 128])
                if p1 == M8 + L and not half:
                    R = TQ - MINI
                    ysum = _cat([yst[ct, MINI:TQ, :] + yst2[ct, MINI:TQ, :] for ct in range(2)])
                    o_ref[pl.ds(g0, R), :] = (x_ref[pl.ds(g0, R), :].astype(F32) + ysum).astype(BF16)
                if tail:
                    nat(y[(p1 - p0) * 8:], TQ, mo(g0 + TQ - MINI, 16))
            items.append((300, fin))
        return items

    def run_step(s, doA, doB, first, fill, pre_chunk=None):
        slots = []
        lag = ALAG if (doA and doB) else 0
        for c in range(NC + lag):
            if doB and c < NC:
                slots.append(("B", c))
            if doA and c >= lag:
                slots.append(("A", c - lag))
        total = sum(c for c, _ in fill)
        acc = lsum = mrun = None
        if doA:
            stage_A_q(s + 1)
        for _, f in first:
            f()
        nsl = len(slots)
        done_cost = 0
        fi = 0
        for i, (kind, c) in enumerate(slots):
            if kind == "B":
                acc, lsum = stage_B_chunk(s, c, acc, lsum)
            else:
                if pre_chunk is not None:
                    pre_chunk(c)
                mrun = stage_A_chunk(s + 1, c, mrun)
            lim = total * min(1.0, (i + 1) / max(nsl - FEND, 1))
            while fi < len(fill) and done_cost + fill[fi][0] / 2 <= lim:
                fill[fi][1]()
                done_cost += fill[fi][0]
                fi += 1
        while fi < len(fill):
            fill[fi][1]()
            fi += 1
        if doA:
            stage_A_fin(mrun)
        if doB:
            stage_B_fin(acc, lsum)

    def prep_c():
        win[...] = _pk(win_ref[...])
        dwc = dwc_ref[...].astype(F32)
        for i in range(K):
            wcb[i] = jnp.broadcast_to(_cat([dwc[i:i + 1, :]] * 2), (8, 2 * D))

    def prep_rest():
        wout[...] = _pk(wout_ref[...])
        wmg[...] = _pk(wm_ref[...])
        wv = wqkv_ref[:, 2 * D:3 * D]
        wvo[...] = _pk(_dot(wv, wo_ref[...]).astype(BF16))
        dwm = dwm_ref[...].astype(F32)
        for i in range(K):
            row = dwm[i:i + 1, :]
            if i == PADK:
                row = row + 1.0
            wmb[i] = jnp.broadcast_to(_cat([row, row]), (8, 4 * D))

    def once(f):
        lax.fori_loop(0, sc_ref[1], lambda i, c: (f(), c)[1], 0)

    def dyn(v):
        return v + sc_ref[0]

    def pre_chunk(c):
        if (c * TK) % TL:
            return
        l = c * TK // TL + 1
        if l >= NL:
            return
        if l in XW:
            x0_copies[XW.index(l)].wait()
            if l == XW[1]:
                wcopy["in"].wait()
                wcopy["dwc"].wait()
                prep_c()
            if l == XW[-1]:
                for name in ("out", "v", "o", "dwm", "mg"):
                    wcopy[name].wait()
                for cp in xr_copies:
                    cp.start()
                prep_rest()
        lnq_chunk(0, l)

    with jax.named_scope("s_pre"):
        x0_copies[0].wait()
        xa0 = ln_chunk(0, 0)
        wcopy["qk"].wait()
        wq = wqkv_ref[:, 0:D]
        wk = wqkv_ref[:, D:2 * D]
        wqk[...] = _pk((_dot_nt(wq, wk) * (D ** -0.5 * LOG2E)).astype(BF16))
        q_chunk(0, 0, xa0)

    nop = (PNOP, lambda: None)
    with jax.named_scope("s_pro"):
        run_step(-1, True, False, [],
                 [nop] + items_C(dyn(0)) + items_C(dyn(1)) + items_D(dyn(0)),
                 pre_chunk=pre_chunk)

    for cp in xr_copies:
        cp.wait()

    def step0():
        ln_items = [(1700, functools.partial(lnq_chunk, b, l)) for b in range(1, B) for l in range(NL)]
        m, d = items_M(dyn(0), 1), items_D(dyn(1))
        if S0ORD == 0:
            fill = ln_items + m + d
        else:
            fill = m[:2] + d[:2] + ln_items[:3] + m[2:] + ln_items[3:6] + d[2:] + ln_items[6:]
        run_step(0, True, True, items_C(dyn(2)), fill)
    with jax.named_scope("s_step0"):
        once(step0)

    def loop_body(s, carry):
        fill = items_M(s - 1, 0) + items_M(s, 1) + items_D(s + 1)
        run_step(s, True, True, items_G(s - 1) + items_C(jnp.minimum(s + 2, NT - 1)), fill)

        @pl.when(s >= 2)
        def _():
            o_copy(pl.multiple_of((s - 2) * TQ, 16), TQ, s - 2).start()
        return carry
    with jax.named_scope("s_loop"):
        lax.fori_loop(1, NT - 1, loop_body, 0)

    with jax.named_scope("s_19"):
        once(lambda: run_step(dyn(NT - 1), False, True, items_G(dyn(NT - 2)),
                              items_M(dyn(NT - 2), 0) + items_M(dyn(NT - 1), 1, last=True)))
        o_copy((NT - 3) * TQ, 2 * TQ - MINI, NT - 3).start()
    with jax.named_scope("s_20"):
        once(lambda: run_step(NT, False, False, items_G(dyn(NT - 1)), items_M(dyn(NT - 1), 0, last=True)))
    with jax.named_scope("s_fin"):
        o_copy((NT - 1) * TQ - MINI, TQ + MINI, NT - 2).start()
        for i in range(NT - 3):
            o_copy(i * TQ, TQ, i).wait()
        o_copy((NT - 3) * TQ, 2 * TQ - MINI, NT - 3).wait()
        o_copy((NT - 1) * TQ - MINI, TQ + MINI, NT - 2).wait()


@jax.jit
def pallas_standalone__conformer_family_e_branchformer__speech_kernel(
    x, w_qkv, w_att_out, w_mlp_in, dw_csgu, w_mlp_out, dw_merge, w_merge,
):
    B, T, D = x.shape
    K = dw_csgu.shape[0]
    TP = -(-T // TL) * TL
    TB = T + 2 * HALO
    NT = B * T // TQ
    x2 = x.reshape(B * T, D)
    kern = functools.partial(_kernel, B=B, T=T, D=D, K=K)
    out = pl.pallas_call(
        kern,
        out_shape=jax.ShapeDtypeStruct((B * T, D), x.dtype),
        in_specs=[pl.BlockSpec(memory_space=pl.ANY)] * 8,
        out_specs=pl.BlockSpec(memory_space=pl.ANY),
        scratch_shapes=[
            pltpu.VMEM((B * T, D), BF16),
            pltpu.VMEM((B * T, D), BF16),
            pltpu.VMEM((D, 3 * D), BF16),
            pltpu.VMEM((D, D), BF16),
            pltpu.VMEM((D, 2 * D), BF16),
            pltpu.VMEM((K, D), BF16),
            pltpu.VMEM((D, D), BF16),
            pltpu.VMEM((K, 2 * D), BF16),
            pltpu.VMEM((2 * D, D), BF16),
            pltpu.VMEM((B, TP // 2, D), U32),
            pltpu.VMEM((TQ, TP), F32),
            pltpu.VMEM((TQ, 128), F32),
            pltpu.VMEM((2, B * T, 128), F32),
            pltpu.VMEM((2, B * TB, 128), F32),
            pltpu.VMEM((4, B * TB, 128), F32),
            pltpu.VMEM((D // 2, D), U32),
            pltpu.VMEM((D // 2, D), U32),
            pltpu.VMEM((D // 2, 2 * D), U32),
            pltpu.VMEM((D // 2, D), U32),
            pltpu.VMEM((D, D), U32),
            pltpu.VMEM((K, 8, 2 * D), F32),
            pltpu.VMEM((K, 8, 4 * D), F32),
            pltpu.VMEM((2, (LD + K - 1) * 8, 128), F32),
            pltpu.VMEM((4, (LE + K - 1) * 8, 128), F32),
            pltpu.VMEM((B * T // 2, D), U32),
            pltpu.VMEM((TQ // 2, D), U32),
            pltpu.VMEM((TQ // 2, D), U32),
            pltpu.VMEM((2, TQ + MINI, 128), F32),
            pltpu.VMEM((2, TQ, 128), F32),
            pltpu.SemaphoreType.DMA((len(XW) + B - 1,)),
            pltpu.SemaphoreType.DMA((8,)),
            pltpu.SemaphoreType.DMA((NT,)),
            pltpu.SMEM((2,), jnp.int32),
        ],
        compiler_params=pltpu.CompilerParams(vmem_limit_bytes=110 * 1024 * 1024),
    )(x2, w_qkv, w_att_out, w_mlp_in, dw_csgu, w_mlp_out, dw_merge, w_merge)
    return out.reshape(B, T, D)
```

```python
import functools
import math

import jax
import jax.numpy as jnp
from jax import lax
import jax.experimental.pallas as pl
import jax.experimental.pallas.tpu as pltpu

F32 = jnp.float32
BF16 = jnp.bfloat16
U32 = jnp.uint32

TQ = 400
TQP = 512
TL = 512
TK = 256
HALO = 16
MINI = 32
LD = TQ // 8
LE = (TQ - MINI) // 8
LOG2E = math.log2(math.e)
NBLK = 8
RC = 208
XW = [0, 1, 2, 4]
AHEAD = 2
INW = 2
ALAG = 4
RPOS = 9
RS = 320
GPOS = 2
PNOP = 3000
S0NOP = 2000


def _ln(xf, eps=1e-5):
    mu = jnp.mean(xf, axis=-1, keepdims=True)
    xc = xf - mu
    var = jnp.mean(xc * xc, axis=-1, keepdims=True)
    return xc * lax.rsqrt(var + eps)


def _gelu(x):
    c0 = math.sqrt(2.0 / math.pi)
    inner = x * (c0 + (c0 * 0.044715) * (x * x))
    hx = 0.5 * x
    return hx + hx * jnp.tanh(inner)


def _dot(a, b):
    return jnp.dot(a, b, preferred_element_type=F32)


def _dot_nt(a, b):
    return lax.dot_general(a, b, (((1,), (1,)), ((), ())), preferred_element_type=F32)


def _cat(planes):
    return jnp.concatenate(planes, axis=-1) if len(planes) > 1 else planes[0]


def _pk(v):
    return pltpu.bitcast(v, U32)


def _up(v):
    return pltpu.bitcast(v, BF16)


def _kernel(x_hbm, wqkv_hbm, wo_hbm, win_hbm, dwc_hbm, wout_hbm, dwm_hbm, wm_hbm,
            o_hbm,
            x_ref, o_ref, wqkv_ref, wo_ref, win_ref, dwc_ref, wout_ref, dwm_ref, wm_ref,
            xa_buf, s_buf, mx_buf, u_buf, g_buf, m_buf, wqk, wvo, win, wout, wmg, wcb, wmb,
            ext_g, ext_m, q_buf, q_cur, a_buf, st_buf, yst, yst2, sem_x, sem_w, sem_o, sc_ref,
            *, B, T, D, K):
    NQ = T // TQ
    NT = B * NQ
    TP = 2 * xa_buf.shape[1]
    TB = T + 2 * HALO
    NC = TP // TK
    NL = TP // TL
    PADK = K // 2
    M8 = MINI // 8
    ORD = list(range(NC - 1))
    ORD.insert(RPOS, NC - 1)

    xgroups = [(XW[i], (XW + [NL])[i + 1]) for i in range(len(XW))]

    def x_copy(b, l0, l1, si):
        g0 = b * T + l0 * TL
        n = min(l1 * TL, T) - l0 * TL
        return pltpu.make_async_copy(x_hbm.at[pl.ds(g0, n), :], x_ref.at[pl.ds(g0, n), :], sem_x.at[si])

    x0_copies = [x_copy(0, l0, l1, i) for i, (l0, l1) in enumerate(xgroups)]
    xr_copies = [x_copy(b, 0, NL, len(xgroups) + b - 1) for b in range(1, B)]

    wlist = [("qk", wqkv_hbm.at[:, pl.ds(0, 2 * D)], wqkv_ref.at[:, pl.ds(0, 2 * D)]),
             ("v", wqkv_hbm.at[:, pl.ds(2 * D, D)], wqkv_ref.at[:, pl.ds(2 * D, D)]),
             ("o", wo_hbm, wo_ref), ("dwc", dwc_hbm, dwc_ref),
             ("dwm", dwm_hbm, dwm_ref), ("in", win_hbm, win_ref), ("out", wout_hbm, wout_ref),
             ("mg", wm_hbm, wm_ref)]
    wcopy = {name: pltpu.make_async_copy(src, dst, sem_w.at[i]) for i, (name, src, dst) in enumerate(wlist)}

    def o_copy(g0, n, i):
        return pltpu.make_async_copy(o_ref.at[pl.ds(g0, n), :], o_hbm.at[pl.ds(g0, n), :], sem_o.at[i])

    wcopy["dwc"].start()
    wcopy["dwm"].start()
    x0_copies[0].start()
    wcopy["qk"].start()
    extra = {INW: ["in"], len(XW) - 1: ["out", "v", "o", "mg"]}

    def gstart(i):
        if i < len(XW):
            x0_copies[i].start()
            for name in extra.get(i, []):
                wcopy[name].start()

    for i in range(1, AHEAD):
        gstart(i)

    sc_ref[0] = 0
    sc_ref[1] = 1

    q_cur[TQ // 2:, :] = jnp.zeros((q_cur.shape[0] - TQ // 2, D), U32)
    for b in range(B):
        xa_buf[b, T // 2:TP // 2, :] = jnp.zeros(((TP - T) // 2, D), U32)
        for ct in range(2):
            g_buf[ct, b * TB:b * TB + HALO, :] = jnp.zeros((HALO, 128), F32)
            g_buf[ct, b * TB + HALO + T:(b + 1) * TB, :] = jnp.zeros((HALO, 128), F32)
        for ct in range(4):
            m_buf[ct, b * TB:b * TB + HALO, :] = jnp.zeros((HALO, 128), F32)
            m_buf[ct, b * TB + HALO + T:(b + 1) * TB, :] = jnp.zeros((HALO, 128), F32)

    wcopy["dwc"].wait()
    wcopy["dwm"].wait()
    dwc = dwc_ref[...].astype(F32)
    dwm = dwm_ref[...].astype(F32)
    for i in range(K):
        wcb[i] = jnp.broadcast_to(_cat([dwc[i:i + 1, :]] * 2), (8, 2 * D))
        row = dwm[i:i + 1, :]
        if i == PADK:
            row = row + 1.0
        wmb[i] = jnp.broadcast_to(_cat([row, row]), (8, 4 * D))

    def batch_of(v, per):
        if isinstance(v, int):
            return v // per
        return sum((v >= per * k).astype(jnp.int32) for k in range(1, B))

    def mo(v, m):
        return v if isinstance(v, int) else pl.multiple_of(v, m)

    def dyn(v):
        return v + sc_ref[0]

    def once(f):
        lax.fori_loop(0, sc_ref[1], lambda i, c: (f(), c)[1], 0)

    def tile_pos(n):
        b = batch_of(n, NQ)
        return b, mo((n - b * NQ) * TQ, 16)

    def ln_rows(b, l):
        r0 = l * TL
        return b * T + r0, r0, min(TL, T - r0)

    def ln_chunk(b, l):
        g0, r0, n = ln_rows(b, l)
        xa = _ln(x_ref[g0:g0 + n, :].astype(F32)).astype(BF16)
        xa_buf[b, r0 // 2:(r0 + n) // 2, :] = _pk(xa)
        return xa

    def q_chunk(b, l, xa):
        g0, r0, n = ln_rows(b, l)
        q_buf[g0 // 2:(g0 + n) // 2, :] = _pk(_dot(xa, _up(wqk[...])).astype(BF16))

    def lnq_chunk(b, l):
        q_chunk(b, l, ln_chunk(b, l))

    def xa_rows(b, start, size):
        half = start // 2 if isinstance(start, int) else pl.multiple_of(lax.shift_right_logical(start, 1), 8)
        return _up(xa_buf[b, pl.ds(half, size // 2), :])

    def relayout(ext, ect, buf, ct, base, L, eo=0):
        for e in range(L + K - 1):
            ext[ect, (eo + e) * 8:(eo + e + 1) * 8, :] = buf[ct, pl.ds(base - PADK + e, 8, stride=L), :]

    def conv_ext(ext, ect, j0, n, wb_ref, wct):
        X = ext[ect, j0 * 8:(j0 + n + K - 1) * 8, :].reshape(-1, 8, 128)
        acc = None
        for i in range(K):
            w = wb_ref[i, :, wct * 128:(wct + 1) * 128]
            term = X[i:i + n] * w[None]
            acc = term if acc is None else acc + term
        return acc.reshape(n * 8, 128)

    def conv_ext_dup(ext, ect, j0, n, wb_ref, wct, wct2):
        return jnp.concatenate(
            [conv_ext(ext, ect, j, 2, wb_ref, wct if (j // 2) % 2 == 0 else wct2)
             for j in range(j0, j0 + n, 2)], axis=0)

    def stage_A_q(n):
        q_cur[0:TQ // 2, :] = q_buf[pl.ds(mo(n * (TQ // 2), 8), TQ // 2), :]

    def stage_A_chunk(n, c, rot=True):
        b, _ = tile_pos(n)
        q = _up(q_cur[0:TQ // 2, :])
        k0 = (ORD[c] if rot else c) * TK
        nfull = min(TK, (T - k0) // 128 * 128)
        parts = []
        if nfull:
            if nfull == 128:
                kk_ = xa_rows(b, k0, nfull)
                s = jnp.concatenate([_dot_nt(q[0:RC], kk_), _dot_nt(q[RC:TQ], kk_)], axis=0)
            else:
                s = _dot_nt(q, xa_rows(b, k0, nfull))
            parts = [s[:, l * 128:(l + 1) * 128] for l in range(nfull // 128)]
        if nfull < TK:
            nr = T - k0 - nfull
            st = _dot_nt(xa_rows(b, k0 + nfull, nr), _up(q_cur[...]))
            st = jnp.concatenate([st, jnp.full((128 - nr, st.shape[1]), -jnp.inf, F32)], axis=0)
            parts.append(st.T[0:TQ, :])
        mrun = st_buf[0] if c > 0 else None
        for l, sl in enumerate(parts):
            kk = k0 + l * 128
            s_buf[:, kk:kk + 128] = sl
            mrun = sl if mrun is None else jnp.maximum(mrun, sl)
        if c < NC - 1:
            st_buf[0] = mrun
        return mrun

    def stage_A_fin(mrun):
        mx = jnp.max(mrun, axis=-1, keepdims=True)
        mx_buf[...] = jnp.broadcast_to(mx, (TQ, 128))

    def stage_B_chunk(n, c, r0=0, r1=TQ):
        b, _ = tile_pos(n)
        mx = mx_buf[r0:r1, :]
        k0 = ORD[c] * TK
        p = jnp.exp2(s_buf[r0:r1, k0:k0 + TK] - _cat([mx] * (TK // 128)))
        lsum = st_buf[1, r0:r1, :] if c > 0 else None
        for l in range(TK // 128):
            pl_ = p[:, l * 128:(l + 1) * 128]
            lsum = pl_ if lsum is None else lsum + pl_
        if c < NC - 1:
            st_buf[1, r0:r1, :] = lsum
        acc = _dot(p.astype(BF16), xa_rows(b, k0, TK))
        if c > 0:
            acc = _cat([st_buf[2, r0:r1, :], st_buf[3, r0:r1, :]]) + acc
        if c < NC - 1:
            st_buf[2, r0:r1, :] = acc[:, 0:128]
            st_buf[3, r0:r1, :] = acc[:, 128:256]
        return acc, lsum

    def stage_B_fin(acc, lsum, r0=0, r1=TQ):
        l = jnp.sum(lsum, axis=-1, keepdims=True)
        a_buf[r0 // 2:r1 // 2, :] = _pk((acc * (1.0 / l)).astype(BF16))

    def items_G(n, r0=0, r1=TQ):
        def f():
            b, rt = tile_pos(n)
            glob = _dot(_up(a_buf[r0 // 2:r1 // 2, :]), _up(wvo[...]))
            base = mo(b * TB + HALO + rt, 16) + r0
            for ct in range(2):
                m_buf[ct, pl.ds(base, r1 - r0), :] = glob[:, ct * 128:(ct + 1) * 128]
        return [(0, f)]

    def items_C(n, tap=None, head=False):
        nn = min(n + 1, NT - 1) if isinstance(n, int) else jnp.minimum(n + 1, NT - 1)
        parts = [[(nn, 0, HALO), (n, 0 if head else HALO, RC)], [(n, RC, TQ)]]
        items = []
        for pi, segs in enumerate(parts):
            def f(pi=pi, segs=segs):
                geo = []
                for (t, o0, o1) in segs:
                    b, r0 = tile_pos(t)
                    geo.append((b, r0 + o0, mo(t * TQ, 16) + o0, mo(b * TB + HALO + r0, 16) + o0, o1 - o0))
                lhs = [xa_rows(b, r, R) for (b, r, _, _, R) in geo]
                lhs = jnp.concatenate(lhs, axis=0) if len(lhs) > 1 else lhs[0]
                hh = _dot(lhs, _up(win[...]))
                if tap is not None and pi == 0:
                    tap(hh[0:8, 0:128])
                h = _gelu(hh)
                g = _ln(h[:, D:])
                o = 0
                for (_, _, gu, gb, R) in geo:
                    for ct in range(2):
                        u_buf[ct, pl.ds(gu, R), :] = h[o:o + R, ct * 128:(ct + 1) * 128]
                        g_buf[ct, pl.ds(gb, R), :] = g[o:o + R, ct * 128:(ct + 1) * 128]
                    o += R
            items.append((25 * 4 * 12, f))
        return items

    def items_D(n):
        b, r0 = tile_pos(n)
        base = mo(b * TB + HALO + r0, 16)
        g0 = mo(n * TQ, 16)
        L = LD
        items = []
        res = {}
        for ct in range(2):
            items.append((80, functools.partial(relayout, ext_g, ct, g_buf, ct, base, L)))
        for j0 in range(0, L, NBLK):
            n_ = min(NBLK, L - j0)
            for ct in range(2):
                def f(j0=j0, n_=n_, ct=ct):
                    gc = conv_ext_dup(ext_g, ct, j0, n_, wcb, ct, ct + 2)
                    u = jnp.concatenate(
                        [u_buf[ct, pl.ds(g0 + j, 8, stride=L), :] for j in range(j0, j0 + n_)], axis=0)
                    res[j0, ct] = u * gc
                items.append((n_ * 64, f))

        def fin():
            z = _cat([jnp.concatenate([res[j0, ct] for j0 in range(0, L, NBLK)], axis=0)
                      for ct in range(2)]).astype(BF16)
            loc = _dot(z, _up(wout[...]))
            for j in range(L):
                for ct in range(2):
                    m_buf[2 + ct, pl.ds(base + j, 8, stride=L), :] = (
                        loc[j * 8:(j + 1) * 8, ct * 128:(ct + 1) * 128])
        items.append((100, fin))
        return items

    def items_M(n, half, last=False, sel=None):
        b, r0 = tile_pos(n)
        g0 = mo(n * TQ, 16)
        gp = max(n * TQ - MINI, 0) if isinstance(n, int) else pl.multiple_of(jnp.maximum(n * TQ - MINI, 0), 16)
        base_p = gp + HALO + batch_of(gp, T) * 2 * HALO
        base = b * TB + HALO + r0
        cts = (2 * half, 2 * half + 1)
        if last:
            La = (RS - MINI) // 8
            segs = [(M8, base_p, gp), (La, base, g0), (LD - La, base + La * 8, g0 + La * 8)]
        else:
            segs = [(M8, base_p, gp), (LE, base, g0)]
        blocks, jb, eo = [], 0, 0
        for (L, bb, gd) in segs:
            blocks.append((jb, L, bb, eo, gd))
            jb += L
            eo += L + K - 1
        if sel is not None:
            blocks = [blocks[i] for i in sel]
        j_lo, j_hi = blocks[0][0], blocks[-1][0] + blocks[-1][1]
        items = []
        res = {}
        for ct in cts:
            def f(ct=ct):
                for (_, L, bb, eo, _) in blocks:
                    relayout(ext_m, ct, m_buf, ct, bb, L, eo)
            items.append((80, f))
        js = []
        for (jb, L, bb, eo, _) in blocks:
            for j0 in range(jb, jb + L, NBLK):
                n_ = min(NBLK, jb + L - j0)
                js.append(j0)
                for ct in cts:
                    def f(j0=j0, n_=n_, ct=ct, e0=eo + j0 - jb):
                        res[j0, ct] = conv_ext_dup(ext_m, ct, e0, n_, wmb, ct, ct + 4)
                    items.append((n_ * 63, f))

        def fin():
            mm = _cat([jnp.concatenate([res[j0, ct] for j0 in js], axis=0)
                       for ct in cts]).astype(BF16)
            y = _dot(mm, _up(wmg[half * (D // 2):(half + 1) * (D // 2), :]))
            yo = TQ if last else 0
            if half:
                yst[yo + j_lo * 8:yo + j_hi * 8, :] = y
                return
            y = y + yst[yo + j_lo * 8:yo + j_hi * 8, :]
            for (jb, L, bb, eo, gd) in blocks:
                for j in range(jb, jb + L):
                    for ct in range(2):
                        yst2[ct, pl.ds(jb * 8 + j - jb, 8, stride=L), :] = (
                            y[(j - j_lo) * 8:(j - j_lo + 1) * 8, ct * 128:(ct + 1) * 128])
            for (jb, L, bb, eo, gd) in blocks:
                yn = _cat([yst2[ct, jb * 8:(jb + L) * 8, :] for ct in range(2)])
                gd = mo(gd, 16)
                o_ref[pl.ds(gd, L * 8), :] = (x_ref[pl.ds(gd, L * 8), :].astype(F32) + yn).astype(BF16)
        items.append((300, fin))
        return items

    def run_step(s, doA, doB, first, fill, pre_chunk=None, post_chunk=None):
        slots = []
        lag = ALAG if (doA and doB) else 0
        for c in range(NC + lag):
            if doB and c < NC:
                slots.append(("B", c))
            if doA and c >= lag:
                slots.append(("A", c - lag))
        total = sum(c for c, _ in fill)
        acc = lsum = mrun = None
        if doA:
            stage_A_q(s + 1)
        for _, f in first:
            f()
        nsl = len(slots)
        done_cost = 0
        fi = 0
        for i, (kind, c) in enumerate(slots):
            if kind == "B":
                acc, lsum = stage_B_chunk(s, c)
            else:
                if pre_chunk is not None:
                    pre_chunk(c)
                mrun = stage_A_chunk(s + 1, c, rot=pre_chunk is None)
                if post_chunk is not None:
                    post_chunk(c)
            lim = total * (i + 1) / nsl
            while fi < len(fill) and done_cost + fill[fi][0] / 2 <= lim:
                fill[fi][1]()
                done_cost += fill[fi][0]
                fi += 1
        while fi < len(fill):
            fill[fi][1]()
            fi += 1
        if doA:
            stage_A_fin(mrun)
        if doB:
            stage_B_fin(acc, lsum)

    def pre_chunk(c):
        if (c * TK) % TL:
            return
        l = c * TK // TL + 1
        if l not in XW:
            return
        i = XW.index(l)
        x0_copies[i].wait()
        gstart(i + AHEAD)
        for name in extra.get(i, []):
            wcopy[name].wait()
        if i == INW:
            win[...] = _pk(win_ref[...])
        if i == len(XW) - 1:
            for cp in xr_copies:
                cp.start()
            wout[...] = _pk(wout_ref[...])
            wmg[...] = _pk(wm_ref[...])
            wvo[...] = _pk(_dot(wqkv_ref[:, 2 * D:3 * D], wo_ref[...]).astype(BF16))

    def post_chunk(c):
        if ((c + 1) * TK) % TL:
            return
        l = (c + 1) * TK // TL
        if l < NL:
            lnq_chunk(0, l)

    x0_copies[0].wait()
    wcopy["qk"].wait()
    gstart(AHEAD)
    xa0 = ln_chunk(0, 0)
    wqk[...] = _pk((_dot_nt(wqkv_ref[:, 0:D], wqkv_ref[:, D:2 * D]) * (D ** -0.5 * LOG2E)).astype(BF16))
    q_chunk(0, 0, xa0)

    def nop(c):
        return [(c, lambda: None)]

    run_step(-1, True, False, [],
             nop(PNOP) + items_C(dyn(0), head=True) + items_D(dyn(0)),
             pre_chunk=pre_chunk, post_chunk=post_chunk)

    for cp in xr_copies:
        cp.wait()

    def step0():
        ln_items = [(1700, functools.partial(lnq_chunk, b, l)) for b in range(1, B) for l in range(NL)]

        def tap(v):
            m_buf[2, pl.ds(mo(B * TB + dyn(0) * 8, 8), 8), :] = v
        run_step(0, True, True, items_C(dyn(1), tap),
                 nop(S0NOP) + ln_items + items_M(dyn(0), 1) + items_D(dyn(1)))
    once(step0)

    def loop_body(s, carry):
        fill = items_M(s - 1, 0) + items_M(s, 1) + items_D(s + 1)
        run_step(s, True, True, items_G(s - 1) + items_C(s + 1), fill)

        @pl.when(s >= 2)
        def _():
            o_copy(pl.multiple_of((s - 2) * TQ, 16), TQ, s - 2).start()
        return carry
    lax.fori_loop(1, NT - 1, loop_body, 0)

    cut = (NT - 1) * TQ + RS - MINI
    tail_copies = [o_copy((NT - 3) * TQ, 2 * TQ - MINI, NT - 3),
                   o_copy(cut - RS, RS, NT - 1),
                   o_copy(cut, NT * TQ - cut, NT - 2)]

    def step_last():
        n = dyn(NT - 1)
        for _, f in items_G(dyn(NT - 2)):
            f()
        fill1 = (items_M(n, 1, last=True) + items_M(dyn(NT - 2), 0)
                 + [(0, lambda: tail_copies[0].start())])
        fill2 = items_G(n, 0, RS) + items_M(n, 0, last=True, sel=(0, 1))
        for (r0, r1, fill, c0) in ((0, RS, fill1, 0), (RS, TQ, fill2, GPOS)):
            total = sum(c for c, _ in fill)
            done, fi = 0, 0
            for c in range(NC):
                acc, lsum = stage_B_chunk(n, c, r0, r1)
                while (fi < len(fill) and c >= c0
                       and done + fill[fi][0] / 2 <= total * (c + 1 - c0) / (NC - c0)):
                    fill[fi][1]()
                    done += fill[fi][0]
                    fi += 1
            while fi < len(fill):
                fill[fi][1]()
                fi += 1
            stage_B_fin(acc, lsum, r0, r1)

    once(step_last)
    tail_copies[1].start()
    once(lambda: run_step(NT, False, False, items_G(dyn(NT - 1), RS, TQ),
                          items_M(dyn(NT - 1), 0, last=True, sel=(2,))))
    tail_copies[2].start()
    for i in range(NT - 3):
        o_copy(i * TQ, TQ, i).wait()
    for cp in tail_copies:
        cp.wait()


@jax.jit
def pallas_standalone__conformer_family_e_branchformer__speech_kernel(
    x, w_qkv, w_att_out, w_mlp_in, dw_csgu, w_mlp_out, dw_merge, w_merge,
):
    B, T, D = x.shape
    K = dw_csgu.shape[0]
    TP = -(-T // TL) * TL
    TB = T + 2 * HALO
    NT = B * T // TQ
    assert D == 256 and T % TQ == 0 and T % 16 == 0 and K // 2 < HALO and K % 2 == 1
    assert TP - T < 128 and TP // TL > XW[-1] and NT >= 4
    x2 = x.reshape(B * T, D)
    kern = functools.partial(_kernel, B=B, T=T, D=D, K=K)
    out = pl.pallas_call(
        kern,
        out_shape=jax.ShapeDtypeStruct((B * T, D), x.dtype),
        in_specs=[pl.BlockSpec(memory_space=pl.ANY)] * 8,
        out_specs=pl.BlockSpec(memory_space=pl.ANY),
        scratch_shapes=[
            pltpu.VMEM((B * T, D), BF16),
            pltpu.VMEM((B * T, D), BF16),
            pltpu.VMEM((D, 3 * D), BF16),
            pltpu.VMEM((D, D), BF16),
            pltpu.VMEM((D, 2 * D), BF16),
            pltpu.VMEM((K, D), BF16),
            pltpu.VMEM((D, D), BF16),
            pltpu.VMEM((K, 2 * D), BF16),
            pltpu.VMEM((2 * D, D), BF16),
            pltpu.VMEM((B, TP // 2, D), U32),
            pltpu.VMEM((TQ, TP), F32),
            pltpu.VMEM((TQ, 128), F32),
            pltpu.VMEM((2, NT * TQ, 128), F32),
            pltpu.VMEM((2, B * TB + 32, 128), F32),
            pltpu.VMEM((4, B * TB + 32, 128), F32),
            pltpu.VMEM((D // 2, D), U32),
            pltpu.VMEM((D // 2, D), U32),
            pltpu.VMEM((D // 2, 2 * D), U32),
            pltpu.VMEM((D // 2, D), U32),
            pltpu.VMEM((D, D), U32),
            pltpu.VMEM((K, 8, 2 * D), F32),
            pltpu.VMEM((K, 8, 4 * D), F32),
            pltpu.VMEM((2, (LD + K - 1) * 8, 128), F32),
            pltpu.VMEM((4, TQ + MINI + 3 * (K - 1) * 8, 128), F32),
            pltpu.VMEM((B * T // 2, D), U32),
            pltpu.VMEM((TQP // 2, D), U32),
            pltpu.VMEM((TQ // 2, D), U32),
            pltpu.VMEM((4, TQ, 128), F32),
            pltpu.VMEM((2 * TQ + MINI, D), F32),
            pltpu.VMEM((2, TQ + MINI, 128), F32),
            pltpu.SemaphoreType.DMA((len(XW) + B - 1,)),
            pltpu.SemaphoreType.DMA((8,)),
            pltpu.SemaphoreType.DMA((NT,)),
            pltpu.SMEM((2,), jnp.int32),
        ],
        compiler_params=pltpu.CompilerParams(vmem_limit_bytes=110 * 1024 * 1024),
    )(x2, w_qkv, w_att_out, w_mlp_in, dw_csgu, w_mlp_out, dw_merge, w_merge)
    return out.reshape(B, T, D)
```

```python
import functools
import math

import jax
import jax.numpy as jnp
from jax import lax
import jax.experimental.pallas as pl
import jax.experimental.pallas.tpu as pltpu

F32 = jnp.float32
BF16 = jnp.bfloat16
U32 = jnp.uint32

TQ = 400
TQP = 512
TL = 512
TK = 256
HALO = 16
MINI = 32
LD = TQ // 8
LE = (TQ - MINI) // 8
LOG2E = math.log2(math.e)
NBLK = 8
RC = 208
XW = [0, 1, 2, 4]
AHEAD = 2
INW = 2
ALAG = 4
RPOS = 9
RS = 272
PNOP = 3000
S0NOP = 2000


def _ln(xf, eps=1e-5):
    mu = jnp.mean(xf, axis=-1, keepdims=True)
    xc = xf - mu
    var = jnp.mean(xc * xc, axis=-1, keepdims=True)
    return xc * lax.rsqrt(var + eps)


def _gelu(x):
    c0 = math.sqrt(2.0 / math.pi)
    inner = x * (c0 + (c0 * 0.044715) * (x * x))
    hx = 0.5 * x
    return hx + hx * jnp.tanh(inner)


def _dot(a, b):
    return jnp.dot(a, b, preferred_element_type=F32)


def _dot_nt(a, b):
    return lax.dot_general(a, b, (((1,), (1,)), ((), ())), preferred_element_type=F32)


def _cat(planes):
    return jnp.concatenate(planes, axis=-1) if len(planes) > 1 else planes[0]


def _pk(v):
    return pltpu.bitcast(v, U32)


def _up(v):
    return pltpu.bitcast(v, BF16)


def _kernel(x_hbm, wqkv_hbm, wo_hbm, win_hbm, dwc_hbm, wout_hbm, dwm_hbm, wm_hbm,
            o_hbm,
            x_ref, o_ref, wqkv_ref, wo_ref, win_ref, dwc_ref, wout_ref, dwm_ref, wm_ref,
            xa_buf, s_buf, mx_buf, u_buf, g_buf, m_buf, wqk, wvo, win, wout, wmg, wcb, wmb,
            ext_g, ext_m, q_buf, q_cur, a_buf, st_buf, yst, yst2, sem_x, sem_w, sem_o, sc_ref,
            *, B, T, D, K):
    NQ = T // TQ
    NT = B * NQ
    TP = 2 * xa_buf.shape[1]
    TB = T + 2 * HALO
    NC = TP // TK
    NL = TP // TL
    PADK = K // 2
    M8 = MINI // 8
    ORD = list(range(NC - 1))
    ORD.insert(RPOS, NC - 1)

    xgroups = [(XW[i], (XW + [NL])[i + 1]) for i in range(len(XW))]

    def x_copy(b, l0, l1, si):
        g0 = b * T + l0 * TL
        n = min(l1 * TL, T) - l0 * TL
        return pltpu.make_async_copy(x_hbm.at[pl.ds(g0, n), :], x_ref.at[pl.ds(g0, n), :], sem_x.at[si])

    x0_copies = [x_copy(0, l0, l1, i) for i, (l0, l1) in enumerate(xgroups)]
    xr_copies = [x_copy(b, 0, NL, len(xgroups) + b - 1) for b in range(1, B)]

    wlist = [("qk", wqkv_hbm.at[:, pl.ds(0, 2 * D)], wqkv_ref.at[:, pl.ds(0, 2 * D)]),
             ("v", wqkv_hbm.at[:, pl.ds(2 * D, D)], wqkv_ref.at[:, pl.ds(2 * D, D)]),
             ("o", wo_hbm, wo_ref), ("dwc", dwc_hbm, dwc_ref),
             ("dwm", dwm_hbm, dwm_ref), ("in", win_hbm, win_ref), ("out", wout_hbm, wout_ref),
             ("mg", wm_hbm, wm_ref)]
    wcopy = {name: pltpu.make_async_copy(src, dst, sem_w.at[i]) for i, (name, src, dst) in enumerate(wlist)}

    def o_copy(g0, n, i):
        return pltpu.make_async_copy(o_ref.at[pl.ds(g0, n), :], o_hbm.at[pl.ds(g0, n), :], sem_o.at[i])

    wcopy["dwc"].start()
    wcopy["dwm"].start()
    x0_copies[0].start()
    wcopy["qk"].start()
    extra = {INW: ["in"], len(XW) - 1: ["out", "v", "o", "mg"]}

    def gstart(i):
        if i < len(XW):
            x0_copies[i].start()
            for name in extra.get(i, []):
                wcopy[name].start()

    for i in range(1, AHEAD):
        gstart(i)

    sc_ref[0] = 0
    sc_ref[1] = 1

    q_cur[TQ // 2:, :] = jnp.zeros((q_cur.shape[0] - TQ // 2, D), U32)
    for b in range(B):
        xa_buf[b, T // 2:TP // 2, :] = jnp.zeros(((TP - T) // 2, D), U32)
        for ct in range(2):
            g_buf[ct, b * TB:b * TB + HALO, :] = jnp.zeros((HALO, 128), F32)
            g_buf[ct, b * TB + HALO + T:(b + 1) * TB, :] = jnp.zeros((HALO, 128), F32)
        for ct in range(4):
            m_buf[ct, b * TB:b * TB + HALO, :] = jnp.zeros((HALO, 128), F32)
            m_buf[ct, b * TB + HALO + T:(b + 1) * TB, :] = jnp.zeros((HALO, 128), F32)

    wcopy["dwc"].wait()
    wcopy["dwm"].wait()
    dwc = dwc_ref[...].astype(F32)
    dwm = dwm_ref[...].astype(F32)
    for i in range(K):
        wcb[i] = jnp.broadcast_to(_cat([dwc[i:i + 1, :]] * 2), (8, 2 * D))
        row = dwm[i:i + 1, :]
        if i == PADK:
            row = row + 1.0
        wmb[i] = jnp.broadcast_to(_cat([row, row]), (8, 4 * D))

    def batch_of(v, per):
        if isinstance(v, int):
            return v // per
        return sum((v >= per * k).astype(jnp.int32) for k in range(1, B))

    def mo(v, m):
        return v if isinstance(v, int) else pl.multiple_of(v, m)

    def dyn(v):
        return v + sc_ref[0]

    def once(f):
        lax.fori_loop(0, sc_ref[1], lambda i, c: (f(), c)[1], 0)

    def tile_pos(n):
        b = batch_of(n, NQ)
        return b, mo((n - b * NQ) * TQ, 16)

    def ln_rows(b, l):
        r0 = l * TL
        return b * T + r0, r0, min(TL, T - r0)

    def ln_chunk(b, l):
        g0, r0, n = ln_rows(b, l)
        xa = _ln(x_ref[g0:g0 + n, :].astype(F32)).astype(BF16)
        xa_buf[b, r0 // 2:(r0 + n) // 2, :] = _pk(xa)
        return xa

    def q_chunk(b, l, xa):
        g0, r0, n = ln_rows(b, l)
        q_buf[g0 // 2:(g0 + n) // 2, :] = _pk(_dot(xa, _up(wqk[...])).astype(BF16))

    def lnq_chunk(b, l):
        q_chunk(b, l, ln_chunk(b, l))

    def xa_rows(b, start, size):
        half = start // 2 if isinstance(start, int) else pl.multiple_of(lax.shift_right_logical(start, 1), 8)
        return _up(xa_buf[b, pl.ds(half, size // 2), :])

    def relayout(ext, ect, buf, ct, base, L, eo=0):
        b0 = base - PADK
        for e in range(L + K - 1):
            ext[ect, (eo + e) * 8:(eo + e + 1) * 8, :] = buf[ct, pl.ds(b0 + e, 8, stride=L), :]

    def conv_ext_dup(ext, ect, j0, n, wb_ref, wct, wct2):
        X = ext[ect, j0 * 8:(j0 + n + K - 1) * 8, :].reshape(-1, 8, 128)
        pat = [((j0 + j) // 2) % 2 for j in range(n)]
        acc = None
        for i in range(K):
            w2 = [wb_ref[i:i + 1, :, c * 128:(c + 1) * 128] for c in (wct, wct2)]
            term = X[i:i + n] * jnp.concatenate([w2[p] for p in pat], axis=0)
            acc = term if acc is None else acc + term
        return acc.reshape(n * 8, 128)

    def stage_A_q(n):
        q_cur[0:TQ // 2, :] = q_buf[pl.ds(mo(n * (TQ // 2), 8), TQ // 2), :]

    def stage_A_chunk(n, c, rot=True):
        b, _ = tile_pos(n)
        q = _up(q_cur[0:TQ // 2, :])
        k0 = (ORD[c] if rot else c) * TK
        nfull = min(TK, (T - k0) // 128 * 128)
        parts = []
        if nfull:
            if nfull == 128:
                kk_ = xa_rows(b, k0, nfull)
                s = jnp.concatenate([_dot_nt(q[0:RC], kk_), _dot_nt(q[RC:TQ], kk_)], axis=0)
            else:
                s = _dot_nt(q, xa_rows(b, k0, nfull))
            parts = [s[:, l * 128:(l + 1) * 128] for l in range(nfull // 128)]
        if nfull < TK:
            nr = T - k0 - nfull
            st = _dot_nt(xa_rows(b, k0 + nfull, nr), _up(q_cur[...]))
            st = jnp.concatenate([st, jnp.full((128 - nr, st.shape[1]), -jnp.inf, F32)], axis=0)
            parts.append(st.T[0:TQ, :])
        mrun = st_buf[0] if c > 0 else None
        for l, sl in enumerate(parts):
            kk = k0 + l * 128
            s_buf[:, kk:kk + 128] = sl
            mrun = sl if mrun is None else jnp.maximum(mrun, sl)
        if c < NC - 1:
            st_buf[0] = mrun
        return mrun

    def stage_A_fin(mrun):
        mx = jnp.max(mrun, axis=-1, keepdims=True)
        mx_buf[...] = jnp.broadcast_to(mx, (TQ, 128))

    def stage_B_chunk(n, c, r0=0, r1=TQ):
        b, _ = tile_pos(n)
        mx = mx_buf[r0:r1, :]
        k0 = ORD[c] * TK
        p = jnp.exp2(s_buf[r0:r1, k0:k0 + TK] - _cat([mx] * (TK // 128)))
        lsum = st_buf[1, r0:r1, :] if c > 0 else None
        for l in range(TK // 128):
            pl_ = p[:, l * 128:(l + 1) * 128]
            lsum = pl_ if lsum is None else lsum + pl_
        if c < NC - 1:
            st_buf[1, r0:r1, :] = lsum
        acc = _dot(p.astype(BF16), xa_rows(b, k0, TK))
        if c > 0:
            acc = _cat([st_buf[2, r0:r1, :], st_buf[3, r0:r1, :]]) + acc
        if c < NC - 1:
            st_buf[2, r0:r1, :] = acc[:, 0:128]
            st_buf[3, r0:r1, :] = acc[:, 128:256]
        return acc, lsum

    def stage_B_fin(acc, lsum, r0=0, r1=TQ):
        l = jnp.sum(lsum, axis=-1, keepdims=True)
        a_buf[r0 // 2:r1 // 2, :] = _pk((acc * (1.0 / l)).astype(BF16))

    def items_G(n, r0=0, r1=TQ):
        def f():
            b, rt = tile_pos(n)
            glob = _dot(_up(a_buf[r0 // 2:r1 // 2, :]), _up(wvo[...]))
            base = mo(b * TB + HALO + rt, 16) + r0
            for ct in range(2):
                m_buf[ct, pl.ds(base, r1 - r0), :] = glob[:, ct * 128:(ct + 1) * 128]
        return [(0, f)]

    def items_C(n, tap=None, head=False):
        nn = min(n + 1, NT - 1) if isinstance(n, int) else jnp.minimum(n + 1, NT - 1)
        parts = [[(nn, 0, HALO), (n, 0 if head else HALO, RC)], [(n, RC, TQ)]]
        items = []
        for pi, segs in enumerate(parts):
            def f(pi=pi, segs=segs):
                geo = []
                for (t, o0, o1) in segs:
                    b, r0 = tile_pos(t)
                    geo.append((b, r0 + o0, mo(t * TQ, 16) + o0, mo(b * TB + HALO + r0, 16) + o0, o1 - o0))
                lhs = [xa_rows(b, r, R) for (b, r, _, _, R) in geo]
                lhs = jnp.concatenate(lhs, axis=0) if len(lhs) > 1 else lhs[0]
                hh = _dot(lhs, _up(win[...]))
                if tap is not None and pi == 0:
                    tap(hh[0:8, 0:128])
                h = _gelu(hh)
                g = _ln(h[:, D:])
                o = 0
                for (_, _, gu, gb, R) in geo:
                    for ct in range(2):
                        u_buf[ct, pl.ds(gu, R), :] = h[o:o + R, ct * 128:(ct + 1) * 128]
                        g_buf[ct, pl.ds(gb, R), :] = g[o:o + R, ct * 128:(ct + 1) * 128]
                    o += R
            items.append((25 * 4 * 12, f))
        return items

    def items_D(n):
        b, r0 = tile_pos(n)
        base = mo(b * TB + HALO + r0, 16)
        g0 = mo(n * TQ, 16)
        L = LD
        items = []
        res = {}
        for ct in range(2):
            items.append((80, functools.partial(relayout, ext_g, ct, g_buf, ct, base, L)))
        for j0 in range(0, L, NBLK):
            n_ = min(NBLK, L - j0)
            for ct in range(2):
                def f(j0=j0, n_=n_, ct=ct):
                    gc = conv_ext_dup(ext_g, ct, j0, n_, wcb, ct, ct + 2)
                    u = jnp.concatenate(
                        [u_buf[ct, pl.ds(g0 + j, 8, stride=L), :] for j in range(j0, j0 + n_)], axis=0)
                    res[j0, ct] = u * gc
                items.append((n_ * 64, f))

        def fin():
            z = _cat([jnp.concatenate([res[j0, ct] for j0 in range(0, L, NBLK)], axis=0)
                      for ct in range(2)]).astype(BF16)
            loc = _dot(z, _up(wout[...]))
            for j in range(L):
                for ct in range(2):
                    m_buf[2 + ct, pl.ds(base + j, 8, stride=L), :] = (
                        loc[j * 8:(j + 1) * 8, ct * 128:(ct + 1) * 128])
        items.append((100, fin))
        return items

    def items_M(n, half, last=False, sel=None):
        b, r0 = tile_pos(n)
        g0 = mo(n * TQ, 16)
        gp = max(n * TQ - MINI, 0) if isinstance(n, int) else pl.multiple_of(jnp.maximum(n * TQ - MINI, 0), 16)
        base_p = gp + HALO + batch_of(gp, T) * 2 * HALO
        base = b * TB + HALO + r0
        cts = (2 * half, 2 * half + 1)
        if last:
            La = (RS - MINI) // 8
            segs = [(M8, base_p, gp), (La, base, g0), (LD - La, base + La * 8, g0 + La * 8)]
        else:
            segs = [(M8, base_p, gp), (LE, base, g0)]
        blocks, jb, eo = [], 0, 0
        for (L, bb, gd) in segs:
            blocks.append((jb, L, bb, eo, gd))
            jb += L
            eo += L + K - 1
        if sel is not None:
            blocks = [blocks[i] for i in sel]
        j_lo, j_hi = blocks[0][0], blocks[-1][0] + blocks[-1][1]
        items = []
        res = {}
        for ct in cts:
            def f(ct=ct):
                for (_, L, bb, eo, _) in blocks:
                    relayout(ext_m, ct, m_buf, ct, bb, L, eo)
            items.append((80, f))
        js = []
        for (jb, L, bb, eo, _) in blocks:
            for j0 in range(jb, jb + L, NBLK):
                n_ = min(NBLK, jb + L - j0)
                js.append(j0)
                for ct in cts:
                    def f(j0=j0, n_=n_, ct=ct, e0=eo + j0 - jb):
                        res[j0, ct] = conv_ext_dup(ext_m, ct, e0, n_, wmb, ct, ct + 4)
                    items.append((n_ * 63, f))

        def fin():
            mm = _cat([jnp.concatenate([res[j0, ct] for j0 in js], axis=0)
                       for ct in cts]).astype(BF16)
            y = _dot(mm, _up(wmg[half * (D // 2):(half + 1) * (D // 2), :]))
            yo = TQ if last else 0
            if half:
                yst[yo + j_lo * 8:yo + j_hi * 8, :] = y
                return
            y = y + yst[yo + j_lo * 8:yo + j_hi * 8, :]
            for (jb, L, bb, eo, gd) in blocks:
                for j in range(jb, jb + L):
                    for ct in range(2):
                        yst2[ct, pl.ds(jb * 8 + j - jb, 8, stride=L), :] = (
                            y[(j - j_lo) * 8:(j - j_lo + 1) * 8, ct * 128:(ct + 1) * 128])
            for (jb, L, bb, eo, gd) in blocks:
                yn = _cat([yst2[ct, jb * 8:(jb + L) * 8, :] for ct in range(2)])
                gd = mo(gd, 16)
                o_ref[pl.ds(gd, L * 8), :] = (x_ref[pl.ds(gd, L * 8), :].astype(F32) + yn).astype(BF16)
        items.append((300, fin))
        return items

    def run_step(s, doA, doB, first, fill, pre_chunk=None, post_chunk=None):
        slots = []
        lag = ALAG if (doA and doB) else 0
        for c in range(NC + lag):
            if doB and c < NC:
                slots.append(("B", c))
            if doA and c >= lag:
                slots.append(("A", c - lag))
        total = sum(c for c, _ in fill)
        acc = lsum = mrun = None
        if doA:
            stage_A_q(s + 1)
        for _, f in first:
            f()
        nsl = len(slots)
        done_cost = 0
        fi = 0
        for i, (kind, c) in enumerate(slots):
            if kind == "B":
                acc, lsum = stage_B_chunk(s, c)
            else:
                if pre_chunk is not None:
                    pre_chunk(c)
                mrun = stage_A_chunk(s + 1, c, rot=pre_chunk is None)
                if post_chunk is not None:
                    post_chunk(c)
            lim = total * (i + 1) / nsl
            while fi < len(fill) and done_cost + fill[fi][0] / 2 <= lim:
                fill[fi][1]()
                done_cost += fill[fi][0]
                fi += 1
        while fi < len(fill):
            fill[fi][1]()
            fi += 1
        if doA:
            stage_A_fin(mrun)
        if doB:
            stage_B_fin(acc, lsum)

    def pre_chunk(c):
        if (c * TK) % TL:
            return
        l = c * TK // TL + 1
        if l not in XW:
            return
        i = XW.index(l)
        x0_copies[i].wait()
        gstart(i + AHEAD)
        for name in extra.get(i, []):
            wcopy[name].wait()
        if i == INW:
            win[...] = _pk(win_ref[...])
        if i == len(XW) - 1:
            for cp in xr_copies:
                cp.start()
            wout[...] = _pk(wout_ref[...])
            wmg[...] = _pk(wm_ref[...])
            wvo[...] = _pk(_dot(wqkv_ref[:, 2 * D:3 * D], wo_ref[...]).astype(BF16))

    def post_chunk(c):
        if ((c + 1) * TK) % TL:
            return
        l = (c + 1) * TK // TL
        if l < NL:
            lnq_chunk(0, l)

    x0_copies[0].wait()
    wcopy["qk"].wait()
    gstart(AHEAD)
    xa0 = ln_chunk(0, 0)
    wqk[...] = _pk((_dot_nt(wqkv_ref[:, 0:D], wqkv_ref[:, D:2 * D]) * (D ** -0.5 * LOG2E)).astype(BF16))
    q_chunk(0, 0, xa0)

    def nop(c):
        return [(c, lambda: None)]

    run_step(-1, True, False, [],
             nop(PNOP) + items_C(dyn(0), head=True) + items_D(dyn(0)),
             pre_chunk=pre_chunk, post_chunk=post_chunk)

    for cp in xr_copies:
        cp.wait()

    def step0():
        ln_items = [(1700, functools.partial(lnq_chunk, b, l)) for b in range(1, B) for l in range(NL)]

        def tap(v):
            m_buf[2, pl.ds(mo(B * TB + dyn(0) * 8, 8), 8), :] = v
        run_step(0, True, True, items_C(dyn(1), tap),
                 nop(S0NOP) + ln_items + items_M(dyn(0), 1) + items_D(dyn(1)))
    once(step0)

    def loop_body(s, carry):
        fill = items_M(s - 1, 0) + items_M(s, 1) + items_D(s + 1)
        run_step(s, True, True, items_G(s - 1) + items_C(s + 1), fill)

        @pl.when(s >= 2)
        def _():
            o_copy(pl.multiple_of((s - 2) * TQ, 16), TQ, s - 2).start()
        return carry
    lax.fori_loop(1, NT - 1, loop_body, 0)

    cut = (NT - 1) * TQ + RS - MINI
    tail_copies = [o_copy((NT - 3) * TQ, 2 * TQ - MINI, NT - 3),
                   o_copy(cut - RS, RS, NT - 1),
                   o_copy(cut, NT * TQ - cut, NT - 2)]

    def b_range(r0, r1, first, fill):
        for _, f in first:
            f()
        total = sum(c for c, _ in fill)
        done, fi = 0, 0
        n = dyn(NT - 1)
        for c in range(NC):
            acc, lsum = stage_B_chunk(n, c, r0, r1)
            while fi < len(fill) and done + fill[fi][0] / 2 <= total * (c + 1) / NC:
                fill[fi][1]()
                done += fill[fi][0]
                fi += 1
        while fi < len(fill):
            fill[fi][1]()
            fi += 1
        stage_B_fin(acc, lsum, r0, r1)

    once(lambda: b_range(0, RS, items_G(dyn(NT - 2)),
                         items_M(dyn(NT - 1), 1, last=True) + items_M(dyn(NT - 2), 0)
                         + [(0, lambda: tail_copies[0].start())]))
    once(lambda: b_range(RS, TQ, items_G(dyn(NT - 1), 0, RS),
                         items_M(dyn(NT - 1), 0, last=True, sel=(0, 1))))
    tail_copies[1].start()
    once(lambda: run_step(NT, False, False, items_G(dyn(NT - 1), RS, TQ),
                          items_M(dyn(NT - 1), 0, last=True, sel=(2,))))
    tail_copies[2].start()
    for i in range(NT - 3):
        o_copy(i * TQ, TQ, i).wait()
    for cp in tail_copies:
        cp.wait()


@jax.jit
def pallas_standalone__conformer_family_e_branchformer__speech_kernel(
    x, w_qkv, w_att_out, w_mlp_in, dw_csgu, w_mlp_out, dw_merge, w_merge,
):
    B, T, D = x.shape
    K = dw_csgu.shape[0]
    TP = -(-T // TL) * TL
    TB = T + 2 * HALO
    NT = B * T // TQ
    assert D == 256 and T % TQ == 0 and T % 16 == 0 and K // 2 < HALO and K % 2 == 1
    assert TP - T < 128 and TP // TL > XW[-1] and NT >= 4
    x2 = x.reshape(B * T, D)
    kern = functools.partial(_kernel, B=B, T=T, D=D, K=K)
    out = pl.pallas_call(
        kern,
        out_shape=jax.ShapeDtypeStruct((B * T, D), x.dtype),
        in_specs=[pl.BlockSpec(memory_space=pl.ANY)] * 8,
        out_specs=pl.BlockSpec(memory_space=pl.ANY),
        scratch_shapes=[
            pltpu.VMEM((B * T, D), BF16),
            pltpu.VMEM((B * T, D), BF16),
            pltpu.VMEM((D, 3 * D), BF16),
            pltpu.VMEM((D, D), BF16),
            pltpu.VMEM((D, 2 * D), BF16),
            pltpu.VMEM((K, D), BF16),
            pltpu.VMEM((D, D), BF16),
            pltpu.VMEM((K, 2 * D), BF16),
            pltpu.VMEM((2 * D, D), BF16),
            pltpu.VMEM((B, TP // 2, D), U32),
            pltpu.VMEM((TQ, TP), F32),
            pltpu.VMEM((TQ, 128), F32),
            pltpu.VMEM((2, NT * TQ + 64, 128), F32),
            pltpu.VMEM((2, B * TB + 64, 128), F32),
            pltpu.VMEM((4, B * TB + 64, 128), F32),
            pltpu.VMEM((D // 2, D), U32),
            pltpu.VMEM((D // 2, D), U32),
            pltpu.VMEM((D // 2, 2 * D), U32),
            pltpu.VMEM((D // 2, D), U32),
            pltpu.VMEM((D, D), U32),
            pltpu.VMEM((K, 8, 2 * D), F32),
            pltpu.VMEM((K, 8, 4 * D), F32),
            pltpu.VMEM((2, (LD + K - 1) * 8, 128), F32),
            pltpu.VMEM((4, TQ + MINI + 3 * (K - 1) * 8, 128), F32),
            pltpu.VMEM((B * T // 2, D), U32),
            pltpu.VMEM((TQP // 2, D), U32),
            pltpu.VMEM((TQ // 2, D), U32),
            pltpu.VMEM((4, TQ, 128), F32),
            pltpu.VMEM((2 * TQ + MINI, D), F32),
            pltpu.VMEM((2, TQ + MINI + 48, 128), F32),
            pltpu.SemaphoreType.DMA((len(XW) + B - 1,)),
            pltpu.SemaphoreType.DMA((8,)),
            pltpu.SemaphoreType.DMA((NT,)),
            pltpu.SMEM((2,), jnp.int32),
        ],
        compiler_params=pltpu.CompilerParams(vmem_limit_bytes=110 * 1024 * 1024),
    )(x2, w_qkv, w_att_out, w_mlp_in, dw_csgu, w_mlp_out, dw_merge, w_merge)
    return out.reshape(B, T, D)
```
